```python
import os as _os
_os.environ.setdefault("JAX_PLATFORMS", "cpu")
import jax
import jax.numpy as jnp

def _softmax(x, axis=-1):
    return jax.nn.softmax(x, axis=axis)
def _gelu(x):
    return jax.nn.gelu(x, approximate=True)
def _silu(x):
    return jax.nn.silu(x)
def _sigmoid(x):
    return jax.nn.sigmoid(x)
def _layernorm(x, axis=-1, eps=1e-5):
    m = jnp.mean(x, axis=axis, keepdims=True)
    v = jnp.var(x, axis=axis, keepdims=True)
    return (x - m) / jnp.sqrt(v + eps)
def _scatter_add(tgt, idx, src, axis=0):
    return tgt.at[idx].add(src)
def _segment_sum(src, seg, n):
    return jax.ops.segment_sum(src, seg, n)
class _Rng:
    def __init__(self, key):
        self._k = key
    def _next(self):
        self._k, sub = jax.random.split(self._k)
        return sub
    def normal(self, shape):
        return jax.random.normal(self._next(), shape, dtype=jnp.bfloat16)
    def randint(self, lo, hi, shape):
        return jax.random.randint(self._next(), shape, lo, hi, dtype=jnp.int32)
    def uniform(self, shape, lo=0.0, hi=1.0):
        return jax.random.uniform(self._next(), shape, jnp.bfloat16, lo, hi)
    def permutation(self, n):
        return jax.random.permutation(self._next(), n)


kernel_name = 'standalone__gqa_block_cached__sampling'

def setup_inputs():
    _rng = _Rng(jax.random.key(int.from_bytes(__import__("os").urandom(4), "little")))
    _w = (lambda a: (lambda t: t.astype(jnp.bfloat16) if jnp.issubdtype(t.dtype, jnp.floating) else t)(jnp.asarray(a)))
    B, Sq, D = 32, 16, 1024
    Hq, Hkv, Sk, Dh = 32, 4, 2048, 128
    assert Hq % Hkv == 0, (Hq, Hkv)
    return {
        "x": _w((lambda *s: _rng.normal(s) * 0.8)(B, Sq, D)),
        "k_cache": _w((lambda *s: _rng.normal(s) * 0.8)(B, Hkv, Sk, Dh)),
        "v_cache": _w((lambda *s: _rng.normal(s) * 0.05)(B, Hkv, Sk, Dh)),
        "wq": _w((lambda *s: _rng.normal(s) * 0.8)(D, Hq * Dh) * (D ** -0.5)),
        "wo": _w((lambda *s: _rng.normal(s) * 0.05)(Hq * Dh, D) * ((Hq * Dh) ** -0.5)),
    }

def reference(x, k_cache, v_cache, wq, wo):
    B, Sq, D = x.shape
    Hq, Dh = 32, 128
    Hkv = k_cache.shape[1]
    rep = Hq // Hkv
    q = (lambda x, *d: x.transpose(*d))((x @ wq).reshape(B, Sq, Hq, Dh), 0, 2, 1, 3)
    k = jnp.repeat(k_cache, rep, axis=1)
    v = jnp.repeat(v_cache, rep, axis=1)
    scores = jnp.einsum("bhqd,bhkd->bhqk", q, k) * (Dh ** -0.5)
    p = _softmax(scores, axis=-1)
    o = jnp.einsum("bhqk,bhkd->bhqd", p, v)
    return (lambda x, *d: x.transpose(*d))(o, 0, 2, 1, 3).reshape(B, Sq, Hq * Dh) @ wo
```

```python
import contextlib
import numpy as np
import jax
import jax.numpy as jnp
from jax import lax
from jax.experimental import pallas as pl
from jax.experimental.pallas import tpu as pltpu

PATS = {
    "cross4": [(0, 3), (1, 2), (2, 1), (3, 0)],
    "within4": [(0, 0), (0, 1), (0, 2), (0, 3)],
    "2x2": [(0, 1), (0, 3), (1, 0), (1, 2)],
    "2x2c": [(0, 2), (0, 3), (1, 0), (1, 1)],
}


def make_kernel(NS=8, LU=14, NODMA=0, DBC=1, PAT="cross4", SA="WD1mDq2DD3", SB="WD1mDq2DoD3", SC="WD1mDo2DoD3",
                SD="WD1mDh2DhD3", WP=1, XP=32, WQP=64, SCOPES=0, PROI=1, FLAGS="", NOCOMP=0, PERMW=1, **kw):
    ROWS = 128
    scope = (lambda n: jax.named_scope(n)) if SCOPES else (lambda n: contextlib.nullcontext())
    pat = PATS[PAT]
    maxoff = max(p[0] for p in pat)

    def f(x, k_cache, v_cache, wq, wo):
        B, Sq, D = x.shape
        _, Hkv, Sk, Dh = k_cache.shape
        Hq = wq.shape[1] // Dh
        rep = Hq // Hkv
        M = rep * Sq
        GW = rep * Dh
        R = B * Sq
        NSLAB = B * Hkv
        GB = 128 // Sq
        NG = NSLAB // GB
        GPH = B // GB
        c = float(Dh ** -0.5) * float(np.log2(np.e))
        x2 = x.reshape(R, D)
        k2 = k_cache.reshape(NSLAB * Sk, Dh)
        v2 = v_cache.reshape(NSLAB * Sk, Dh)
        QR = Sk // 4
        isint = lambda v: isinstance(v, int)
        mo = lambda v, m: v if isint(v) else pl.multiple_of(v, m)

        def kern(x_hbm, k_hbm, v_hbm, wq_hbm, wo_hbm, out_hbm,
                 xb, wqb, wob, kb, vb, qs, os_, acc, outb, kv_sem, w_sem, o_sem):
            def row0(s):
                return ((s & (B - 1)) * Hkv + (s >> 5)) * Sk

            def slot_of(s):
                return s & (NS - 1)

            def chunk(which, s, quarter, cc):
                src = (k_hbm, v_hbm)[which]
                dst = (kb, vb)[which]
                slot = slot_of(s)
                off = quarter * QR + cc * ROWS
                return pltpu.make_async_copy(src.at[pl.ds(mo(row0(s) + off, ROWS), ROWS)],
                                             dst.at[slot, pl.ds(mo(off, ROWS), ROWS)],
                                             kv_sem.at[which, slot])

            def unit_tc(t, cc, guard):
                if NODMA: return
                for (so, qu) in pat:
                    sl = t + so
                    if isint(sl):
                        if 0 <= sl < NSLAB:
                            for which in range(2):
                                chunk(which, sl, qu, cc).start(priority=which)
                    elif guard:
                        @pl.when(sl < NSLAB)
                        def _():
                            for which in range(2):
                                chunk(which, sl, qu, cc).start(priority=which)
                    else:
                        for which in range(2):
                            chunk(which, sl, qu, cc).start(priority=which)

            def unit(s, k, guard):
                n = LU + k
                unit_tc(s + n // 4, n % 4, guard)

            def wait_kv(which, s):
                if NODMA: return
                buf = (kb, vb)[which]
                slot = slot_of(s)
                pltpu.make_async_copy(buf.at[slot], buf.at[slot], kv_sem.at[which, slot]).wait()

            def wpiece(s, k, nk):
                rr = 128 // nk
                mat = s >> 3
                r = mo((s & 7) * 128 + k * rr, rr)
                @pl.when(jnp.logical_and((mat & 1) == 0, s < 56))
                def _():
                    h = mat >> 1
                    pltpu.make_async_copy(wo_hbm.at[pl.ds(mo(h * GW + r, rr), rr)], wob.at[h, pl.ds(r, rr)],
                                          w_sem.at[1 + Hkv + h]).start(priority=k % 2)
                @pl.when(jnp.logical_and((mat & 1) == 1, s < 56))
                def _():
                    h = (mat + 1) >> 1
                    pltpu.make_async_copy(wq_hbm.at[pl.ds(r, rr), pl.ds(mo(h * GW, GW), GW)], wqb.at[h, pl.ds(r, rr)],
                                          w_sem.at[1 + h]).start(priority=k % 2)

            def wait_wq(h):
                pltpu.make_async_copy(wqb.at[h], wqb.at[h], w_sem.at[1 + h]).wait()

            def wait_wo(h):
                pltpu.make_async_copy(wob.at[h], wob.at[h], w_sem.at[1 + Hkv + h]).wait()

            def qpiece(G, j):
                h = G >> 2
                r0 = mo((G & 3) * 128, 128)
                co = mo(j * Dh, Dh)
                ro = mo(j * Sq, Sq)
                q = jnp.dot(xb[pl.ds(r0, 128), :], wqb[h, :, pl.ds(co, Dh)], preferred_element_type=jnp.float32) * c
                q = q.astype(jnp.bfloat16)
                for bb in range(GB):
                    qs[G * GB + bb, pl.ds(ro, Sq), :] = q[bb * Sq:(bb + 1) * Sq, :]

            def opiece(G, j, nrow=128, ncol=Dh, rsub=0):
                h = G >> 2
                r0 = mo((G & 3) * 128 + rsub, nrow)
                par = G & 1
                co = mo(j * ncol, ncol)
                a = jnp.dot(os_[par, pl.ds(rsub, nrow), :], wob[h, :, pl.ds(co, ncol)], preferred_element_type=jnp.float32)
                a = a + acc[pl.ds(r0, nrow), pl.ds(co, ncol)]
                acc[pl.ds(r0, nrow), pl.ds(co, ncol)] = a
                outb[pl.ds(r0, nrow), pl.ds(co, ncol)] = a.astype(jnp.bfloat16)

            def attn1(s):
                return lax.dot_general(qs[s], kb[slot_of(s)], (((1,), (1,)), ((), ())), preferred_element_type=jnp.float32)

            def attn2(s, sc, m):
                p = jnp.exp2(sc - m)
                l = jnp.sum(p, axis=1, keepdims=True)
                o = jnp.dot(p.astype(jnp.bfloat16), vb[slot_of(s)], preferred_element_type=jnp.float32)
                return o, l

            def attn3(s, o, l):
                o = (o * (1.0 / l)).astype(jnp.bfloat16)
                par = (s >> 3) & 1
                ro = mo((s & 7) * Sq, Sq)
                for j in range(rep):
                    os_[par, pl.ds(ro, Sq), pl.ds(j * Dh, Dh)] = o[j * Sq:(j + 1) * Sq, :]

            def out_copy(r0, n, sem):
                return pltpu.make_async_copy(outb.at[pl.ds(mo(r0, 64), n)], out_hbm.at[pl.ds(mo(r0, 64), n)], o_sem.at[sem])

            def body(s, sched, guard=False, weights=False, opc=None):
                st = {}
                nd = 0
                no = 0
                nD = sched.count("D")
                assert nD in (0, 4)
                for ch in sched:
                    if NOCOMP and ch in "1m23qoh": continue
                    if ch == "W":
                        wait_kv(0, s); wait_kv(1, s)
                    elif ch == "K":
                        wait_kv(0, s)
                    elif ch == "V":
                        wait_kv(1, s)
                    elif ch == "D":
                        unit(s, nd, guard)
                        if weights and (nd % (4 // WP) == 0):
                            wpiece(s, nd // (4 // WP), WP)
                        nd += 1
                    elif ch == "1":
                        st["sc"] = attn1(s)
                    elif ch == "m":
                        st["m"] = jnp.max(st["sc"], axis=1, keepdims=True)
                    elif ch == "2":
                        st["o"], st["l"] = attn2(s, st["sc"], st["m"])
                    elif ch == "3":
                        attn3(s, st["o"], st["l"])
                    elif ch == "q":
                        s1 = s + 1
                        qpiece(jnp.minimum((s1 >> 3) + 1, NG - 1), s1 & 7)
                    elif ch == "o":
                        opc(s, no)
                        no += 1
                    elif ch == "h":
                        opiece(NG - 1, 2 * (s - (NSLAB - 4)) // 2 * 1 if False else (s - (NSLAB - 4)), nrow=64, ncol=256, rsub=0) if no == 0 else None
                        no += 1
                    else:
                        raise ValueError(ch)

            def loop(name, lo, hi, fn):
                def b_(s, c_):
                    fn(s)
                    return c_
                with scope(name):
                    lax.fori_loop(lo, hi, b_, 0)

            xr = R // XP
            wr = D // WQP
            n0 = LU - 8 if PROI else LU
            with scope("P1_enq"):
                def xl(p, c_):
                    for u in range(2):
                        r = mo((p * 2 + u) * xr, xr)
                        pltpu.make_async_copy(x_hbm.at[pl.ds(r, xr)], xb.at[pl.ds(r, xr)], w_sem.at[0]).start(priority=u)
                    return c_
                lax.fori_loop(0, XP // 2, xl, 0)
                def wl(p, c_):
                    for u in range(2):
                        pi = p * 2 + u
                        pp = (pi & 3) * (WQP // 4) + (pi >> 2) if PERMW else pi
                        r = mo(pp * wr, wr)
                        pltpu.make_async_copy(wq_hbm.at[pl.ds(r, wr), pl.ds(0, GW)], wqb.at[0, pl.ds(r, wr)], w_sem.at[1]).start(priority=u)
                    return c_
                lax.fori_loop(0, WQP // 2, wl, 0)
            with scope("P2_zero"):
                def zl(i, c_):
                    acc[pl.ds(mo(i * 64, 64), 64), :] = jnp.zeros((64, D), acc.dtype)
                    return c_
                lax.fori_loop(0, R // 64, zl, 0)
            with scope("P2_kv"):
                for t in range(-maxoff, 0):
                    for cc in range(4):
                        unit_tc(t, cc, False)
                if n0 > 0:
                    def ul(n, c_):
                        unit_tc(n >> 2, n & 3, False)
                        return c_
                    lax.fori_loop(0, n0, ul, 0)
            with scope("P3_waitxw"):
                pltpu.make_async_copy(xb, xb, w_sem.at[0]).wait()
                wait_wq(0)
            with scope("P4_qproj"):
                def pro(j, c_):
                    if PROI:
                        n = max(n0, 0) + j
                        unit_tc(n >> 2, n & 3, False)
                    if not NOCOMP: qpiece(0, j)
                    return c_
                lax.fori_loop(0, rep, pro, 0)
                if not NOCOMP: qpiece(1, 0)

            def wwaits(s):
                @pl.when(jnp.logical_and((s & 31) == 23, s < 96))
                def _():
                    wait_wq((s >> 5) + 1)
                @pl.when((s & 31) == 8)
                def _():
                    wait_wo(s >> 5)

            loop("LA", 0, 8, lambda s: body(s, SA, weights=True))

            def fB(s):
                wwaits(s)
                body(s, SB, weights=True, opc=lambda s_, k: opiece((s_ >> 3) - 1, s_ & 7))
                @pl.when(jnp.logical_and((s & 7) == 7, s >= 111))
                def _():
                    g = (s >> 3) - 13
                    out_copy(g * 128, 128, g).start()
            loop("LB", 8, 120, fB)

            def fC(s):
                body(s, SC, guard=True, opc=lambda s_, k: opiece(NG - 2, 2 * (s_ - 120) + k))
            loop("LC", 120, 124, fC)
            out_copy(2 * 128, 128, 2).start()

            def fD(s):
                body(s, SD.replace("h", "o"), guard=True,
                     opc=lambda s_, k: opiece(NG - 1, 4 * k + (s_ - 124) if False else (s_ - 124), nrow=64, ncol=256, rsub=0) if k == 0 else None)
            loop("LD", 124, 128, fD)
            with scope("E1_oproj"):
                out_copy(3 * 128, 64, 3).start()
                a = jnp.dot(os_[(NG - 1) & 1, pl.ds(64, 64), :], wob[Hkv - 1], preferred_element_type=jnp.float32)
                a = a + acc[pl.ds(3 * 128 + 64, 64), :]
                outb[pl.ds(3 * 128 + 64, 64), :] = a.astype(jnp.bfloat16)
            with scope("E2_out"):
                out_copy(3 * 128 + 64, 64, 4).start()
                for g in range(3):
                    out_copy(g * 128, 128, g).wait()
                out_copy(3 * 128, 64, 3).wait()
                out_copy(3 * 128 + 64, 64, 4).wait()

        cp = dict(vmem_limit_bytes=100 * 2**20, disable_bounds_checks=bool(DBC))
        if FLAGS:
            cp["flags"] = {k: True for k in FLAGS.split("+")}
        out = pl.pallas_call(
            kern,
            out_shape=jax.ShapeDtypeStruct((R, D), jnp.bfloat16),
            in_specs=[pl.BlockSpec(memory_space=pl.ANY)] * 5,
            out_specs=pl.BlockSpec(memory_space=pl.ANY),
            scratch_shapes=[
                pltpu.VMEM((R, D), jnp.bfloat16),
                pltpu.VMEM((Hkv, D, GW), jnp.bfloat16),
                pltpu.VMEM((Hkv, GW, D), jnp.bfloat16),
                pltpu.VMEM((NS, Sk, Dh), jnp.bfloat16),
                pltpu.VMEM((NS, Sk, Dh), jnp.bfloat16),
                pltpu.VMEM((NSLAB, M, Dh), jnp.bfloat16),
                pltpu.VMEM((2, 128, GW), jnp.bfloat16),
                pltpu.VMEM((R, D), jnp.float32),
                pltpu.VMEM((R, D), jnp.bfloat16),
                pltpu.SemaphoreType.DMA((2, NS)),
                pltpu.SemaphoreType.DMA((1 + 2 * Hkv,)),
                pltpu.SemaphoreType.DMA((5,)),
            ],
            compiler_params=pltpu.CompilerParams(**cp),
        )(x2, k2, v2, wq, wo)
        return out.reshape(B, Sq, D)
    return f


@jax.jit
def pallas_standalone__gqa_block_cached__sampling_kernel(x, k_cache, v_cache, wq, wo):
    return make_kernel()(x, k_cache, v_cache, wq, wo)
```

```python
import contextlib
import numpy as np
import jax
import jax.numpy as jnp
from jax import lax
from jax.experimental import pallas as pl
from jax.experimental.pallas import tpu as pltpu


def make_kernel(NS=8, LU=16, LU2=10, S0=114, SA="DDDDW231", SB="W23DDDD1o", SC="W23DDDD1oo", SD="W231h", SD2="",
                SE1="W231", SE2="VO23", WSTR=8, XP=32, NPRE=160, OUTT=(0, 1, 0, 1), E1S=4,
                NODMA=0, NOCOMP=0, NOE1=0, NOOUT=0, SCOPES=0, SCW=0, DBC=1, DSC=1, FLAGS="", QI=0, ZPOS=1, NQ1=11, ZPP=4, QSTEP=8, **kw):
    ROWS = 128
    scope = (lambda n: jax.named_scope(n)) if SCOPES else (lambda n: contextlib.nullcontext())
    wscope = (lambda n: jax.named_scope(n)) if SCW else (lambda n: contextlib.nullcontext())

    def f(x, k_cache, v_cache, wq, wo):
        B, Sq, D = x.shape
        _, Hkv, Sk, Dh = k_cache.shape
        Hq = wq.shape[1] // Dh
        rep = Hq // Hkv
        M = rep * Sq
        GW = rep * Dh
        R = B * Sq
        NSLAB = B * Hkv
        GB = 128 // Sq
        NG = NSLAB // GB
        c = float(Dh ** -0.5) * float(np.log2(np.e))
        x2 = x.reshape(R, D)
        k2 = k_cache.reshape(NSLAB * Sk, Dh)
        v2 = v_cache.reshape(NSLAB * Sk, Dh)
        isint = lambda v: isinstance(v, int)
        mo = lambda v, m: v if isint(v) else pl.multiple_of(v, m)
        assert LU == 16 and LU2 == 10
        RS = LU - LU2
        N0 = 4 * S0 + LU
        T0 = N0 // 4 - 1
        NTOT = (NSLAB * 16 - 24) // 4
        VTOT = NTOT - N0 - 6
        assert S0 + RS <= 120 and S0 + 2 <= 120
        for sch in (SA, SB, SC):
            assert sch.count("D") == 4 and sch.count("W") == 1 and sch.index("2") < sch.index("1")
        assert 4 * 124 + LU2 - N0 - 6 >= VTOT

        def kern(x_hbm, k_hbm, v_hbm, wq_hbm, wo_hbm, out_hbm,
                 xb, wqb, wob, kb, vb, qs, os_, acc, outb, sbuf, mbuf, kv_sem, w_sem, o_sem):
            def row0(s):
                return ((s & (B - 1)) * Hkv + (s >> 5)) * Sk

            def slot_of(s):
                return s & (NS - 1)

            def chunk(which, s, ch):
                src = (k_hbm, v_hbm)[which]
                dst = (kb, vb)[which]
                slot = slot_of(s)
                off = ch * ROWS
                return pltpu.make_async_copy(src.at[pl.ds(mo(row0(s) + off, ROWS), ROWS)],
                                             dst.at[slot, pl.ds(mo(off, ROWS), ROWS)],
                                             kv_sem.at[which, slot])

            def pair(sl, ch, ok=None):
                def go():
                    for which in range(2):
                        chunk(which, sl, ch).start(priority=which)
                if ok is None:
                    go()
                else:
                    pl.when(ok)(go)

            def unit_tc(t, cc):
                if NODMA: return
                for i in range(4):
                    sl = t + i
                    if isint(sl) and sl < 0:
                        continue
                    pair(sl, (3 - i) * 4 + cc)

            def unit(s, k, mode):
                if NODMA: return
                if mode == 0:
                    n = LU + k
                    unit_tc(s + n // 4, n % 4)
                elif mode == 1:
                    d = s - S0
                    u = 3 * d + k
                    for i in range(4):
                        w = 4 * u + i
                        ge4 = (w >= 4).astype(jnp.int32)
                        ge12 = (w >= 12).astype(jnp.int32)
                        pair(T0 + 1 + ge4 + ge12, w + 12 - 8 * ge4 - 12 * ge12, None if k < 3 else False) if k < 3 else None
                elif mode == 2:
                    d = s - S0
                    v = 4 * d - jnp.minimum(d, RS) + (k - 6)
                    ok = None if k < 3 else d >= RS
                    for i in range(4):
                        pair(T0 + 4 + (v >> 2), 4 * i + (v & 3), ok)
                else:
                    v = 4 * s + (LU2 + k - N0 - 6)
                    for i in range(4):
                        pair(T0 + 4 + (v >> 2), 4 * i + (v & 3))

            def wait_kv(which, s):
                if NODMA: return
                buf = (kb, vb)[which]
                slot = slot_of(s)
                pltpu.make_async_copy(buf.at[slot], buf.at[slot], kv_sem.at[which, slot]).wait()

            LW = int(np.log2(WSTR))

            def wq_piece(w, prio):
                p = w & 127
                r = mo((((p & (WSTR - 1)) * (128 // WSTR)) + (p >> LW)) * 8, 8)
                co = mo((w >> 7) * (2 * GW), 2 * GW)
                pltpu.make_async_copy(wq_hbm.at[pl.ds(r, 8), pl.ds(co, 2 * GW)], wqb.at[pl.ds(r, 8), pl.ds(co, 2 * GW)],
                                      w_sem.at[1 + (w >> 7)]).start(priority=prio)

            def wo_piece(w, prio):
                r = mo((((w & (WSTR - 1)) * (256 // WSTR)) + (w >> LW)) * 16, 16)
                pltpu.make_async_copy(wo_hbm.at[pl.ds(r, 16)], wob.at[pl.ds(r, 16)], w_sem.at[3]).start(priority=prio)

            def wait_wq(half):
                co = mo(half * (2 * GW), 2 * GW)
                pltpu.make_async_copy(wqb.at[:, pl.ds(co, 2 * GW)], wqb.at[:, pl.ds(co, 2 * GW)], w_sem.at[1 + half]).wait()

            def qproj(i):
                h = i >> 2
                jp = i & 3
                co = mo(i * 2 * Dh, 2 * Dh)
                q = jnp.dot(xb[...], wqb[:, pl.ds(co, 2 * Dh)], preferred_element_type=jnp.float32) * c
                q = q.astype(jnp.bfloat16)
                for b in range(B):
                    for e in range(2):
                        qs[h * B + b, pl.ds(mo((jp * 2 + e) * Sq, Sq), Sq), :] = q[b * Sq:(b + 1) * Sq, e * Dh:(e + 1) * Dh]

            def opiece(G, j, nrow=128, ncol=Dh, rsub=0):
                h = G >> 2
                r0 = mo((G & 3) * 128 + rsub, nrow)
                par = G & 1
                co = mo(j * ncol, ncol)
                a = jnp.dot(os_[par, pl.ds(rsub, nrow), :], wob[pl.ds(mo(h * GW, GW), GW), pl.ds(co, ncol)], preferred_element_type=jnp.float32)
                a = a + acc[pl.ds(r0, nrow), pl.ds(co, ncol)]
                acc[pl.ds(r0, nrow), pl.ds(co, ncol)] = a
                outb[pl.ds(r0, nrow), pl.ds(co, ncol)] = a.astype(jnp.bfloat16)

            def attn1(s):
                sc = lax.dot_general(qs[s], kb[slot_of(s)], (((1,), (1,)), ((), ())), preferred_element_type=jnp.float32)
                sbuf[...] = sc
                mbuf[...] = jnp.broadcast_to(jnp.max(sc, axis=1, keepdims=True), (M, Dh))

            def attn2(s):
                mb = mbuf[...]
                p = jnp.exp2(sbuf[...] - jnp.concatenate([mb] * (Sk // Dh), axis=1))
                l = jnp.sum(p, axis=1, keepdims=True)
                o = jnp.dot(p.astype(jnp.bfloat16), vb[slot_of(s)], preferred_element_type=jnp.float32)
                return o, l

            def attn3(s, o, l):
                o = (o * (1.0 / l)).astype(jnp.bfloat16)
                par = (s >> 3) & 1
                ro = mo((s & 7) * Sq, Sq)
                for j in range(rep):
                    os_[par, pl.ds(ro, Sq), pl.ds(j * Dh, Dh)] = o[j * Sq:(j + 1) * Sq, :]

            def out_copy(r0, n, sem, c0=0, nc=D):
                return pltpu.make_async_copy(outb.at[pl.ds(r0, n), pl.ds(c0, nc)], out_hbm.at[pl.ds(r0, n), pl.ds(c0, nc)], o_sem.at[sem])

            def body(s, sched, mode=0, opc=None):
                st = {}
                nd = 0
                no = 0
                for ch in sched:
                    if NOCOMP and ch in "123oh": continue
                    if ch == "W":
                        with wscope("w_W"):
                            wait_kv(0, s + 1); wait_kv(1, s)
                    elif ch == "V":
                        with wscope("w_V"):
                            wait_kv(1, s)
                    elif ch == "K":
                        with wscope("w_K"):
                            wait_kv(0, s + 1)
                    elif ch == "X":
                        with wscope("w_X"):
                            wait_kv(1, s + 1)
                    elif ch == "D":
                        unit(s, nd, mode)
                        nd += 1
                    elif ch == "O":
                        if not NOOUT:
                            for g in range(3):
                                out_copy(g * 128, 128, g).start(priority=OUTT[g])
                        out_copy(3 * 128, 64, 3).start(priority=OUTT[3])
                    elif ch == "1":
                        attn1(s + 1)
                    elif ch == "2":
                        st["o"], st["l"] = attn2(s)
                    elif ch == "3":
                        attn3(s, st["o"], st["l"])
                    elif ch == "o":
                        opc(s, no)
                        no += 1
                    elif ch == "h":
                        opc(s, no)
                        no += 1
                    else:
                        raise ValueError(ch)

            def loop(name, lo, hi, fn):
                def b_(s, c_):
                    fn(s)
                    return c_
                with scope(name):
                    lax.fori_loop(lo, hi, b_, 0)

            xr = R // XP
            with scope("P1"):
                def xl(p, c_):
                    for u in range(2):
                        r = mo((p * 2 + u) * xr, xr)
                        pltpu.make_async_copy(x_hbm.at[pl.ds(r, xr)], xb.at[pl.ds(r, xr)], w_sem.at[0]).start(priority=u)
                    return c_
                lax.fori_loop(0, XP // 2, xl, 0)

                def wl(p, c_):
                    for u in range(2):
                        wq_piece(p * 2 + u, u)
                    return c_

                def zl(i, c_):
                    acc[pl.ds(mo(i * 64, 64), 64), :] = jnp.zeros((64, D), acc.dtype)
                    return c_
                lax.fori_loop(0, 32, wl, 0)
                lax.fori_loop(0, R // 64, zl, 0)
                lax.fori_loop(32, 128, wl, 0)
            with scope("P2_waitx"):
                pltpu.make_async_copy(xb, xb, w_sem.at[0]).wait()

            NZ = 24 + 4 * LU
            ZB = 8 * ZPP
            ZC = (NZ - ZB + (NQ1 - 8) - 1) // (NQ1 - 8)

            def kv_item(z, ok=None):
                if NODMA: return
                ge12 = (z >= 12).astype(jnp.int32)
                ge20 = (z >= 20).astype(jnp.int32)
                y = z - 24
                n = y >> 2
                i = y & 3
                r = z < 24
                pair(jnp.where(r, ge12 + ge20, (n >> 2) + i), jnp.where(r, z - 12 * ge12 - 8 * ge20, (3 - i) * 4 + (n & 3)), ok)

            def fQ(kind):
                def f_(i):
                    def issue():
                        if kind == 0:
                            for e in range(32):
                                wo_piece(32 * i + e, e % 2)
                                if ZPP and e % (32 // ZPP) == (32 // ZPP) - 1: kv_item(ZPP * i + e // (32 // ZPP))
                        else:
                            for e in range(ZC):
                                z = ZB + ZC * (i - 8) + e
                                kv_item(z, None if ZB + ZC * (NQ1 - 9) + e < NZ else z < NZ)
                    if QI & 1: issue()
                    if not NOCOMP:
                        qproj(i)
                    if not (QI & 1): issue()
                return f_
            wait_wq(0)
            loop("LQb", 0, 8, fQ(0))
            wait_wq(1)
            loop("LQc", 8, NQ1, fQ(1))
            with scope("P5_qk0"):
                wait_kv(0, 0)
                if not NOCOMP: attn1(0)

            oB = lambda s_, k: opiece((s_ >> 3) - 1, s_ & 7)
            loop("LA", 0, 8, lambda s: body(s, SA))
            pltpu.make_async_copy(wob, wob, w_sem.at[3]).wait()
            def fBa(s):
                body(s, SB, mode=0, opc=oB)
                if NQ1 < 16 and not NOCOMP:
                    @pl.when(jnp.logical_and((s & (QSTEP - 1)) == QSTEP - 1, s < 8 + QSTEP * (16 - NQ1)))
                    def _():
                        qproj(NQ1 + ((s - 8) // QSTEP))
            loop("LBa", 8, S0, fBa)
            loop("LBt", S0, S0 + 2, lambda s: body(s, SB, mode=1, opc=oB))
            if S0 + 2 < 120:
                loop("LBb", S0 + 2, 120, lambda s: body(s, SB, mode=2, opc=oB))
            loop("LC", 120, 124, lambda s: body(s, SC, mode=(2 if S0 + RS > 120 else 3),
                                               opc=lambda s_, k: opiece(NG - 2, 2 * (s_ - 120) + k)))
            hp = lambda j: opiece(NG - 1, j, nrow=64, ncol=512, rsub=0)
            if SD2:
                with scope("LD"):
                    body(124, SD, opc=lambda s_, k: hp(k))
                    body(125, SD2, opc=lambda s_, k: hp(1))
            else:
                loop("LD", 124, 126, lambda s: body(s, SD, opc=lambda s_, k: hp(s_ - 124)))
            with scope("LE1"):
                body(126, SE1)
            with scope("LE2"):
                body(127, SE2)
            with scope("E1_oproj"):
                wcols = D // E1S
                for e in range(E1S):
                    if not NOE1:
                        a = jnp.dot(os_[(NG - 1) & 1, pl.ds(64, 64), :], wob[pl.ds((Hkv - 1) * GW, GW), pl.ds(e * wcols, wcols)], preferred_element_type=jnp.float32)
                        a = a + acc[pl.ds(3 * 128 + 64, 64), pl.ds(e * wcols, wcols)]
                        outb[pl.ds(3 * 128 + 64, 64), pl.ds(e * wcols, wcols)] = a.astype(jnp.bfloat16)
                    out_copy(3 * 128 + 64, 64, 4, e * wcols, wcols).start(priority=e % 2)
            with scope("E2_out"):
                for g in range(3):
                    if not NOOUT: out_copy(g * 128, 128, g).wait()
                out_copy(3 * 128, 64, 3).wait()
                out_copy(3 * 128 + 64, 64, 4).wait()

        cp = dict(vmem_limit_bytes=100 * 2**20, disable_bounds_checks=bool(DBC))
        if DSC: cp["disable_semaphore_checks"] = True
        if FLAGS:
            cp["flags"] = {k: True for k in FLAGS.split("+")}
        out = pl.pallas_call(
            kern,
            out_shape=jax.ShapeDtypeStruct((R, D), jnp.bfloat16),
            in_specs=[pl.BlockSpec(memory_space=pl.ANY)] * 5,
            out_specs=pl.BlockSpec(memory_space=pl.ANY),
            scratch_shapes=[
                pltpu.VMEM((R, D), jnp.bfloat16),
                pltpu.VMEM((D, Hq * Dh), jnp.bfloat16),
                pltpu.VMEM((Hq * Dh, D), jnp.bfloat16),
                pltpu.VMEM((NS, Sk, Dh), jnp.bfloat16),
                pltpu.VMEM((NS, Sk, Dh), jnp.bfloat16),
                pltpu.VMEM((NSLAB, M, Dh), jnp.bfloat16),
                pltpu.VMEM((2, 128, GW), jnp.bfloat16),
                pltpu.VMEM((R, D), jnp.float32),
                pltpu.VMEM((R, D), jnp.bfloat16),
                pltpu.VMEM((M, Sk), jnp.float32),
                pltpu.VMEM((M, Dh), jnp.float32),
                pltpu.SemaphoreType.DMA((2, NS)),
                pltpu.SemaphoreType.DMA((4,)),
                pltpu.SemaphoreType.DMA((5,)),
            ],
            compiler_params=pltpu.CompilerParams(**cp),
        )(x2, k2, v2, wq, wo)
        return out.reshape(B, Sq, D)
    return f


@jax.jit
def pallas_standalone__gqa_block_cached__sampling_kernel(x, k_cache, v_cache, wq, wo):
    return make_kernel()(x, k_cache, v_cache, wq, wo)
```

```python
import numpy as np

import jax
import jax.numpy as jnp
from jax import lax
from jax.experimental import pallas as pl
from jax.experimental.pallas import tpu as pltpu

CHUNK = 128
NSLOT = 8
LOOK = 16
S_SEQ = 114
NQ_PRO = 11
Q_STEP = 8


def _mo(v, m):
    return v if isinstance(v, int) else pl.multiple_of(v, m)


def _loop(lo, hi, fn):
    def body(i, carry):
        fn(i)
        return carry

    lax.fori_loop(lo, hi, body, 0)


def _kernel(x_hbm, k_hbm, v_hbm, wq_hbm, wo_hbm, out_hbm,
            xb, wqb, wob, kb, vb, qs, os_, acc, outb, sbuf, mbuf,
            kv_sem, w_sem, o_sem, *, dims):
    B, Sq, D, Hq, Hkv, Sk, Dh = dims
    rep = Hq // Hkv
    M = rep * Sq
    GW = rep * Dh
    R = B * Sq
    NSLAB = B * Hkv
    GB = 128 // Sq
    NG = NSLAB // GB
    scale = float(Dh ** -0.5) * float(np.log2(np.e))

    def batch_of(j):
        return ((j & 1) << 4) | (j >> 1)

    def slab_row(s):
        return (batch_of(s & (B - 1)) * Hkv + (s >> 5)) * Sk

    def slot_of(s):
        return s & (NSLOT - 1)

    def start_chunk(s, ch):
        slot = slot_of(s)
        off = ch * CHUNK
        for which, (src, dst) in enumerate(((k_hbm, kb), (v_hbm, vb))):
            pltpu.make_async_copy(
                src.at[pl.ds(_mo(slab_row(s) + off, CHUNK), CHUNK)],
                dst.at[slot, pl.ds(_mo(off, CHUNK), CHUNK)],
                kv_sem.at[which, slot],
            ).start(priority=which)

    def wait_slab(which, s):
        buf = (kb, vb)[which]
        slot = slot_of(s)
        pltpu.make_async_copy(buf.at[slot], buf.at[slot], kv_sem.at[which, slot]).wait()

    N_SEQ = 4 * S_SEQ + LOOK
    T_SEQ = N_SEQ // 4 - 1

    def ramp_item(z):
        ge12 = (z >= 12).astype(jnp.int32)
        ge20 = (z >= 20).astype(jnp.int32)
        y = z - 24
        n, i = y >> 2, y & 3
        start_chunk(jnp.where(z < 24, ge12 + ge20, (n >> 2) + i),
                    jnp.where(z < 24, z - 12 * ge12 - 8 * ge20, (3 - i) * 4 + (n & 3)))

    def unit_interleaved(s, k):
        n = LOOK + k
        for i in range(4):
            start_chunk(s + n // 4 + i, (3 - i) * 4 + n % 4)

    def unit_drain(s, k):
        u = 3 * (s - S_SEQ) + k
        for i in range(4):
            w = 4 * u + i
            ge4 = (w >= 4).astype(jnp.int32)
            ge12 = (w >= 12).astype(jnp.int32)
            start_chunk(T_SEQ + 1 + ge4 + ge12, w + 12 - 8 * ge4 - 12 * ge12)

    def unit_sequential(v):
        for i in range(4):
            start_chunk(T_SEQ + 4 + (v >> 2), 4 * i + (v & 3))

    def start_wq(w, thread):
        p = w & 127
        r = _mo(((p & 7) * 16 + (p >> 3)) * 8, 8)
        co = _mo((w >> 7) * (2 * GW), 2 * GW)
        pltpu.make_async_copy(wq_hbm.at[pl.ds(r, 8), pl.ds(co, 2 * GW)],
                              wqb.at[pl.ds(r, 8), pl.ds(co, 2 * GW)],
                              w_sem.at[1 + (w >> 7)]).start(priority=thread)

    def wait_wq(half):
        co = half * (2 * GW)
        pltpu.make_async_copy(wqb.at[:, pl.ds(co, 2 * GW)], wqb.at[:, pl.ds(co, 2 * GW)],
                              w_sem.at[1 + half]).wait()

    def start_wo(w, thread):
        r = _mo(((w & 7) * 32 + (w >> 3)) * 16, 16)
        pltpu.make_async_copy(wo_hbm.at[pl.ds(r, 16)], wob.at[pl.ds(r, 16)],
                              w_sem.at[3]).start(priority=thread)

    def q_piece(i):
        h, jp = i >> 2, i & 3
        q = jnp.dot(xb[...], wqb[:, pl.ds(_mo(i * 2 * Dh, 2 * Dh), 2 * Dh)],
                    preferred_element_type=jnp.float32) * scale
        q = q.astype(jnp.bfloat16)
        for j in range(B):
            b = batch_of(j)
            for e in range(2):
                qs[h * B + j, pl.ds(_mo((jp * 2 + e) * Sq, Sq), Sq), :] = (
                    q[b * Sq:(b + 1) * Sq, e * Dh:(e + 1) * Dh])

    def o_piece(g, j, nrow=128, ncol=Dh, row0=0):
        co = _mo(j * ncol, ncol)
        a = jnp.dot(os_[g & 1, pl.ds(row0, nrow), :],
                    wob[pl.ds(_mo((g >> 2) * GW, GW), GW), pl.ds(co, ncol)],
                    preferred_element_type=jnp.float32)
        for i in range(row0 // Sq, (row0 + nrow) // Sq):
            r = _mo(batch_of((g & 3) * GB + i) * Sq, Sq)
            ai = a[i * Sq - row0:(i + 1) * Sq - row0, :] + acc[pl.ds(r, Sq), pl.ds(co, ncol)]
            acc[pl.ds(r, Sq), pl.ds(co, ncol)] = ai
            outb[pl.ds(r, Sq), pl.ds(co, ncol)] = ai.astype(jnp.bfloat16)

    def scores(s):
        sc = lax.dot_general(qs[s], kb[slot_of(s)], (((1,), (1,)), ((), ())),
                             preferred_element_type=jnp.float32)
        sbuf[...] = sc
        mbuf[...] = jnp.broadcast_to(jnp.max(sc, axis=1, keepdims=True), (M, Dh))

    def attend(s):
        mb = mbuf[...]
        p = jnp.exp2(sbuf[...] - jnp.concatenate([mb] * (Sk // Dh), axis=1))
        l = jnp.sum(p, axis=1, keepdims=True)
        o = jnp.dot(p.astype(jnp.bfloat16), vb[slot_of(s)], preferred_element_type=jnp.float32)
        o = (o * (1.0 / l)).astype(jnp.bfloat16)
        ro = _mo((s & (GB - 1)) * Sq, Sq)
        for j in range(rep):
            os_[(s >> 3) & 1, pl.ds(ro, Sq), pl.ds(j * Dh, Dh)] = o[j * Sq:(j + 1) * Sq, :]

    def wait_iter(s):
        wait_slab(0, s + 1)
        wait_slab(1, s)

    EARLY = ((0, 112), (112, 112), (256, 112), (368, 112))
    LATE = ((224, 32), (480, 32))

    def out_copy(r, n, sem):
        return pltpu.make_async_copy(outb.at[pl.ds(r, n)], out_hbm.at[pl.ds(r, n)], o_sem.at[sem])

    def x_step(p):
        for t in range(2):
            r = _mo((2 * p + t) * 16, 16)
            pltpu.make_async_copy(x_hbm.at[pl.ds(r, 16)], xb.at[pl.ds(r, 16)],
                                  w_sem.at[0]).start(priority=t)

    def wq_step(p):
        for t in range(2):
            start_wq(2 * p + t, t)

    def zero_step(i):
        acc[pl.ds(_mo(i * 64, 64), 64), :] = jnp.zeros((64, D), acc.dtype)

    _loop(0, R // 32, x_step)
    _loop(0, 32, wq_step)
    _loop(0, R // 64, zero_step)
    _loop(32, 128, wq_step)
    pltpu.make_async_copy(xb, xb, w_sem.at[0]).wait()

    N_INIT = 24 + 4 * LOOK
    Z_PER = -(-(N_INIT - 32) // (NQ_PRO - 8))

    def q_step_a(i):
        q_piece(i)
        for e in range(32):
            start_wo(32 * i + e, e % 2)
            if e % 8 == 7:
                ramp_item(4 * i + e // 8)

    def q_step_b(i):
        q_piece(i)
        for e in range(Z_PER):
            z = 32 + Z_PER * (i - 8) + e
            if 32 + Z_PER * (NQ_PRO - 9) + e < N_INIT:
                ramp_item(z)
            else:
                pl.when(z < N_INIT)(lambda z=z: ramp_item(z))

    wait_wq(0)
    _loop(0, 8, q_step_a)
    wait_wq(1)
    _loop(8, NQ_PRO, q_step_b)

    wait_slab(0, 0)
    scores(0)

    def prev_piece(s):
        o_piece((s >> 3) - 1, s & 7)

    def it_first(s):
        for k in range(4):
            unit_interleaved(s, k)
        wait_iter(s)
        attend(s)
        scores(s + 1)

    def it_main(s):
        wait_iter(s)
        attend(s)
        for k in range(4):
            unit_interleaved(s, k)
        scores(s + 1)
        prev_piece(s)

        @pl.when(jnp.logical_and((s & (Q_STEP - 1)) == Q_STEP - 1, s < 8 + Q_STEP * (16 - NQ_PRO)))
        def _():
            q_piece(NQ_PRO + ((s - 8) // Q_STEP))

    def it_drain(s):
        wait_iter(s)
        attend(s)
        for k in range(3):
            unit_drain(s, k)
        scores(s + 1)
        prev_piece(s)

    def it_seq3(s):
        wait_iter(s)
        attend(s)
        for k in range(3):
            unit_sequential(3 * (s - S_SEQ) + (k - 6))
        scores(s + 1)
        prev_piece(s)

    def it_seq4(s):
        wait_iter(s)
        attend(s)
        for k in range(4):
            unit_sequential(4 * s + (k + 4 - N_SEQ))
        scores(s + 1)
        for k in range(2):
            o_piece(NG - 2, 2 * (s - 120) + k)

    assert Q_STEP == 8 and S_SEQ + 6 == 120
    _loop(0, 8, it_first)
    pltpu.make_async_copy(wob, wob, w_sem.at[3]).wait()
    _loop(8, S_SEQ, it_main)
    _loop(S_SEQ, S_SEQ + 2, it_drain)
    _loop(S_SEQ + 2, 120, it_seq3)
    _loop(120, 124, it_seq4)

    wait_iter(124)
    attend(124)
    scores(125)
    for j in range(2):
        o_piece(NG - 1, j, nrow=64, ncol=D // 2, row0=0)
    for s in (125, 126):
        wait_iter(s)
        attend(s)
        scores(s + 1)

    wait_slab(1, 127)
    for n, (r, nr) in enumerate(EARLY):
        out_copy(r, nr, n).start(priority=n % 2)
    attend(127)
    o_piece(NG - 1, 0, nrow=64, ncol=D, row0=64)
    for n, (r, nr) in enumerate(LATE):
        out_copy(r, nr, len(EARLY) + n).start(priority=n % 2)
    for n, (r, nr) in enumerate(EARLY + LATE):
        out_copy(r, nr, n).wait()


@jax.jit
def pallas_standalone__gqa_block_cached__sampling_kernel(
    x: jax.Array,
    k_cache: jax.Array,
    v_cache: jax.Array,
    wq: jax.Array,
    wo: jax.Array,
):
    B, Sq, D = x.shape
    _, Hkv, Sk, Dh = k_cache.shape
    Hq = wq.shape[1] // Dh
    assert (B, Sq, D, Hq, Hkv, Sk, Dh) == (32, 16, 1024, 32, 4, 2048, 128)
    assert v_cache.shape == k_cache.shape and wo.shape == (Hq * Dh, D)
    R = B * Sq
    bf16 = jnp.bfloat16

    def kernel(*refs):
        _kernel(*refs, dims=(B, Sq, D, Hq, Hkv, Sk, Dh))

    out = pl.pallas_call(
        kernel,
        out_shape=jax.ShapeDtypeStruct((R, D), bf16),
        in_specs=[pl.BlockSpec(memory_space=pl.ANY)] * 5,
        out_specs=pl.BlockSpec(memory_space=pl.ANY),
        scratch_shapes=[
            pltpu.VMEM((R, D), bf16),
            pltpu.VMEM((D, Hq * Dh), bf16),
            pltpu.VMEM((Hq * Dh, D), bf16),
            pltpu.VMEM((NSLOT, Sk, Dh), bf16),
            pltpu.VMEM((NSLOT, Sk, Dh), bf16),
            pltpu.VMEM((B * Hkv, 128, Dh), bf16),
            pltpu.VMEM((2, 128, Hq // Hkv * Dh), bf16),
            pltpu.VMEM((R, D), jnp.float32),
            pltpu.VMEM((R, D), bf16),
            pltpu.VMEM((128, Sk), jnp.float32),
            pltpu.VMEM((128, Dh), jnp.float32),
            pltpu.SemaphoreType.DMA((2, NSLOT)),
            pltpu.SemaphoreType.DMA((4,)),
            pltpu.SemaphoreType.DMA((6,)),
        ],
        compiler_params=pltpu.CompilerParams(
            vmem_limit_bytes=64 * 2**20,
            disable_bounds_checks=True,
            disable_semaphore_checks=True,
        ),
    )(
        x.reshape(R, D),
        k_cache.reshape(B * Hkv * Sk, Dh),
        v_cache.reshape(B * Hkv * Sk, Dh),
        wq,
        wo,
    )
    return out.reshape(B, Sq, D)
```
